```python
import jax
import jax.numpy as jnp

def _softmax(x, axis=-1):
    return jax.nn.softmax(x, axis=axis)
def _gelu(x):
    return jax.nn.gelu(x, approximate=True)
def _silu(x):
    return jax.nn.silu(x)
def _sigmoid(x):
    return jax.nn.sigmoid(x)
def _layernorm(x, axis=-1, eps=1e-5):
    m = jnp.mean(x, axis=axis, keepdims=True)
    v = jnp.var(x, axis=axis, keepdims=True)
    return (x - m) / jnp.sqrt(v + eps)
def _scatter_add(tgt, idx, src, axis=0):
    return tgt.at[idx].add(src)
def _segment_sum(src, seg, n):
    return jax.ops.segment_sum(src, seg, n)
class _Rng:
    def __init__(self, key):
        self._k = key
    def _next(self):
        self._k, sub = jax.random.split(self._k)
        return sub
    def normal(self, shape):
        return jax.random.normal(self._next(), shape, dtype=jnp.bfloat16)
    def randint(self, lo, hi, shape):
        return jax.random.randint(self._next(), shape, lo, hi, dtype=jnp.int32)
    def uniform(self, shape, lo=0.0, hi=1.0):
        return jax.random.uniform(self._next(), shape, jnp.bfloat16, lo, hi)
    def permutation(self, n):
        return jax.random.permutation(self._next(), n)


kernel_name = 'standalone__fused_io_aware_attn__prompt'

def setup_inputs():
    _rng = _Rng(jax.random.key(int.from_bytes(__import__("os").urandom(4), "little")))
    _w = (lambda a: (lambda t: t.astype(jnp.bfloat16) if jnp.issubdtype(t.dtype, jnp.floating) else t)(jnp.asarray(a)))
    B, H, S = 2, 32, 2048
    Dh = max(1, 1024 // 32)
    return {
        "q": _w((lambda *s: _rng.normal(s) * 0.05)(B, H, S, Dh)),
        "k": _w((lambda *s: _rng.normal(s) * 0.05)(B, H, S, Dh)),
        "v": _w((lambda *s: _rng.normal(s) * 0.05)(B, H, S, Dh)),
    }

def reference(q, k, v):
    scale = q.shape[-1] ** -0.5
    s = jnp.einsum('bhqd,bhkd->bhqk', q, k) * scale
    p = _softmax(s, axis=-1)
    return jnp.einsum('bhqk,bhkd->bhqd', p, v)
```

```python
import jax
import jax.numpy as jnp
import jax.experimental.pallas as pl
import jax.experimental.pallas.tpu as pltpu

LOG2E = 1.4426950408889634


@jax.jit
def pallas_standalone__fused_io_aware_attn__prompt_kernel(q: jax.Array, k: jax.Array, v: jax.Array):
    B, H, S, D = q.shape
    N = B * H
    bq = tk = 128
    NS = 8
    NO = 4
    qt = q.transpose(0, 1, 3, 2).reshape(N, D, S)
    kt = k.transpose(0, 1, 3, 2).reshape(N, D, S)
    vt = v.transpose(0, 1, 3, 2).reshape(N, D, S)
    c = D ** -0.5 * LOG2E
    nb = S // bq
    nk = S // tk

    def kern(q_hbm, k_hbm, v_hbm, o_hbm, qb, kb, vb, ob, kT, s_scr, isem, osem):
        def in_copies(h):
            sl = h & (NS - 1)
            return [
                pltpu.make_async_copy(q_hbm.at[h], qb.at[sl], isem.at[0, sl]),
                pltpu.make_async_copy(k_hbm.at[h], kb.at[sl], isem.at[1, sl]),
                pltpu.make_async_copy(v_hbm.at[h], vb.at[sl], isem.at[2, sl]),
            ]

        def out_copy(h):
            sl = h & (NO - 1)
            return pltpu.make_async_copy(ob.at[sl], o_hbm.at[h], osem.at[sl])

        def load_k(h, ks):
            kT[ks, :] = kb[h & (NS - 1), :, ks].T

        def sweep(hq, hv, hk, ms):
            out = []
            for i in range(nb):
                qs = slice(i * bq, (i + 1) * bq)
                if hq is not None:
                    qq = qb[hq & (NS - 1), :, qs]
                for j in range(nk):
                    ks = slice(j * tk, (j + 1) * tk)
                    if hv is not None:
                        s_old = s_scr[i, ks, :]
                    if hq is not None:
                        s = jnp.dot(kT[ks, :], qq, preferred_element_type=jnp.float32)
                        s_scr[i, ks, :] = s
                        mm = s.reshape(tk // 8, 8, bq).max(axis=0)
                        mnew = mm if j == 0 else jnp.maximum(mnew, mm)
                        if i == nb - 1:
                            load_k(hk, ks)
                        if j == nk - 1:
                            out.append(jnp.max(mnew, axis=0, keepdims=True))
                    if hv is not None:
                        p = jnp.exp2((s_old - ms[i]) * c)
                        ps = p.reshape(tk // 8, 8, bq).sum(axis=0)
                        l = ps if j == 0 else l + ps
                        o = jnp.dot(vb[hv & (NS - 1), :, ks], p.astype(vb.dtype),
                                    preferred_element_type=jnp.float32)
                        acc = o if j == 0 else acc + o
                if hv is not None:
                    lsum = jnp.sum(l, axis=0, keepdims=True)
                    ob[hv & (NO - 1), :, qs] = (acc / lsum).astype(ob.dtype)
            return tuple(out)

        def advance_dmas(h):
            @pl.when(h + 2 < N)
            def _():
                for cp in in_copies(h + 2):
                    cp.wait()

            @pl.when(h + 3 < N)
            def _():
                for cp in in_copies(h + 3):
                    cp.start()

            @pl.when(h >= 2)
            def _():
                out_copy(h - 2).wait()

        for cp in in_copies(0) + in_copies(1) + in_copies(2):
            cp.start()
        for cp in in_copies(0):
            cp.wait()
        for j in range(nk):
            load_k(0, slice(j * tk, (j + 1) * tk))
        for cp in in_copies(1):
            cp.wait()
        ms = sweep(0, None, 1, None)
        advance_dmas(0)

        def body(h, ms):
            ms = sweep(h + 1, h, jnp.minimum(h + 2, N - 1), ms)
            out_copy(h).start()
            advance_dmas(h + 1)
            return ms

        ms = jax.lax.fori_loop(0, N - 1, body, ms)

        sweep(None, N - 1, None, ms)
        out_copy(N - 1).start()
        out_copy(N - 2).wait()
        out_copy(N - 1).wait()

    anyspec = pl.BlockSpec(memory_space=pl.ANY)
    o = pl.pallas_call(
        kern,
        in_specs=[anyspec] * 3,
        out_specs=anyspec,
        out_shape=jax.ShapeDtypeStruct((N, D, S), q.dtype),
        scratch_shapes=[
            pltpu.VMEM((NS, D, S), q.dtype),
            pltpu.VMEM((NS, D, S), k.dtype),
            pltpu.VMEM((NS, D, S), v.dtype),
            pltpu.VMEM((NO, D, S), q.dtype),
            pltpu.VMEM((S, D), k.dtype),
            pltpu.VMEM((nb, S, bq), jnp.float32),
            pltpu.SemaphoreType.DMA((3, NS)),
            pltpu.SemaphoreType.DMA((NO,)),
        ],
        compiler_params=pltpu.CompilerParams(
            vmem_limit_bytes=64 << 20, disable_bounds_checks=True),
    )(qt, kt, vt)
    return o.reshape(B, H, D, S).transpose(0, 1, 3, 2)
```
